```python
import os as _os
_os.environ.setdefault("JAX_PLATFORMS", "cpu")
import jax
import jax.numpy as jnp

def _softmax(x, axis=-1):
    return jax.nn.softmax(x, axis=axis)
def _gelu(x):
    return jax.nn.gelu(x, approximate=True)
def _silu(x):
    return jax.nn.silu(x)
def _sigmoid(x):
    return jax.nn.sigmoid(x)
def _layernorm(x, axis=-1, eps=1e-5):
    m = jnp.mean(x, axis=axis, keepdims=True)
    v = jnp.var(x, axis=axis, keepdims=True)
    return (x - m) / jnp.sqrt(v + eps)
def _scatter_add(tgt, idx, src, axis=0):
    return tgt.at[idx].add(src)
def _segment_sum(src, seg, n):
    return jax.ops.segment_sum(src, seg, n)
class _Rng:
    def __init__(self, key):
        self._k = key
    def _next(self):
        self._k, sub = jax.random.split(self._k)
        return sub
    def normal(self, shape):
        return jax.random.normal(self._next(), shape, dtype=jnp.bfloat16)
    def randint(self, lo, hi, shape):
        return jax.random.randint(self._next(), shape, lo, hi, dtype=jnp.int32)
    def uniform(self, shape, lo=0.0, hi=1.0):
        return jax.random.uniform(self._next(), shape, jnp.bfloat16, lo, hi)
    def permutation(self, n):
        return jax.random.permutation(self._next(), n)


kernel_name = 'concat_heads__mha_block_cached__gqa_block_cached__near_ridge'

def setup_inputs():
    _rng = _Rng(jax.random.key(int.from_bytes(__import__("os").urandom(4), "little")))
    _w = (lambda a: (lambda t: t.astype(jnp.bfloat16) if jnp.issubdtype(t.dtype, jnp.floating) else t)(jnp.asarray(a)))
    def _A_setup():
        B, Sq, D = 16, 160, 512
        H, Sk, Dh = 32, 1024, 128
        return {
            "x": _w((lambda *s: _rng.normal(s) * 0.8)(B, Sq, D)),
            "k_cache": _w((lambda *s: _rng.normal(s) * 0.8)(B, H, Sk, Dh)),
            "v_cache": _w((lambda *s: _rng.normal(s) * 0.05)(B, H, Sk, Dh)),
            "wq": _w((lambda *s: _rng.normal(s) * 0.8)(D, H * Dh) * (D ** -0.5)),
            "wo": _w((lambda *s: _rng.normal(s) * 0.05)(H * Dh, D) * ((H * Dh) ** -0.5)),
        }
    _A_in = _A_setup()

    def _B_setup():
        B, Sq, D = 16, 160, 512
        Hq, Hkv, Sk, Dh = 32, 32, 1024, 128
        assert Hq % Hkv == 0, (Hq, Hkv)
        return {
            "x": _w((lambda *s: _rng.normal(s) * 0.8)(B, Sq, D)),
            "k_cache": _w((lambda *s: _rng.normal(s) * 0.8)(B, Hkv, Sk, Dh)),
            "v_cache": _w((lambda *s: _rng.normal(s) * 0.05)(B, Hkv, Sk, Dh)),
            "wq": _w((lambda *s: _rng.normal(s) * 0.8)(D, Hq * Dh) * (D ** -0.5)),
            "wo": _w((lambda *s: _rng.normal(s) * 0.05)(Hq * Dh, D) * ((Hq * Dh) ** -0.5)),
        }
    _B_in = _B_setup()

    return {
        "A_x": _A_in["x"],
        "A_k_cache": _A_in["k_cache"],
        "A_v_cache": _A_in["v_cache"],
        "A_wq": _A_in["wq"],
        "A_wo": _A_in["wo"],
        "B_x": _B_in["x"],
        "B_k_cache": _B_in["k_cache"],
        "B_v_cache": _B_in["v_cache"],
        "B_wq": _B_in["wq"],
        "B_wo": _B_in["wo"],
    }

def reference(A_x, A_k_cache, A_v_cache, A_wq, A_wo, B_x, B_k_cache, B_v_cache, B_wq, B_wo):
    def _A_ref(x, k_cache, v_cache, wq, wo):
        B, Sq, D = x.shape
        H, Dh = 32, 128
        q = (lambda x, *d: x.transpose(*d))((x @ wq).reshape(B, Sq, H, Dh), 0, 2, 1, 3)
        scores = jnp.einsum("bhqd,bhkd->bhqk", q, k_cache) * (Dh ** -0.5)
        p = _softmax(scores, axis=-1)
        o = jnp.einsum("bhqk,bhkd->bhqd", p, v_cache)
        return (lambda x, *d: x.transpose(*d))(o, 0, 2, 1, 3).reshape(B, Sq, H * Dh) @ wo

    def _B_ref(x, k_cache, v_cache, wq, wo):
        B, Sq, D = x.shape
        Hq, Dh = 32, 128
        Hkv = k_cache.shape[1]
        rep = Hq // Hkv
        q = (lambda x, *d: x.transpose(*d))((x @ wq).reshape(B, Sq, Hq, Dh), 0, 2, 1, 3)
        k = jnp.repeat(k_cache, rep, axis=1)
        v = jnp.repeat(v_cache, rep, axis=1)
        scores = jnp.einsum("bhqd,bhkd->bhqk", q, k) * (Dh ** -0.5)
        p = _softmax(scores, axis=-1)
        o = jnp.einsum("bhqk,bhkd->bhqd", p, v)
        return (lambda x, *d: x.transpose(*d))(o, 0, 2, 1, 3).reshape(B, Sq, Hq * Dh) @ wo

    a = _A_ref(A_x, A_k_cache, A_v_cache, A_wq, A_wo)
    b = _B_ref(B_x, B_k_cache, B_v_cache, B_wq, B_wo)
    return jnp.concatenate([a, b], axis=-1)
```

```python
import functools
import jax, jax.numpy as jnp, numpy as np
from jax.experimental import pallas as pl
from jax.experimental.pallas import tpu as pltpu

B, Sq, D, H, Sk, Dh = 16, 160, 512, 32, 1024, 128
LOG2E = 1.4426950408889634
F32, BF16 = jnp.float32, jnp.bfloat16
NT = (((1,), (1,)), ((), ()))

def chunks(T, rows):
    return [(o, min(rows, T - o)) for o in range(0, T, rows)]

def make(G=4, NSLOT=4, P=3, rows=176, dma=True, spread=True, compute=True, flags=None):
    NG = H // G
    NIT = NG * B
    GW = G * Dh
    pattern = []
    for o, r in chunks(Sk, rows):
        j = 0
        for a in range(4):
            for h in range(G):
                pattern.append((a, h, o, r, j % 2)); j += 1

    def kern(ax, ak, av, awq, awo, bx, bk, bv, bwq, bwo, out,
             kv, xb, wq, wo, qb, acc, ob, kvsem, xsem, wsem, osem):
        srcs = (ak, av, bk, bv)

        def kv_start(t, slot, part):
            g = t // B
            b = t % B
            base = b * H + g * G
            for a, h, o, r, prio in part:
                pltpu.make_async_copy(srcs[a].at[base + h, pl.ds(o, r)], kv.at[slot, a, h, pl.ds(o, r)],
                                      kvsem.at[slot]).start(priority=prio)

        def kv_wait(slot):
            pltpu.make_async_copy(kv.at[slot], kv.at[slot], kvsem.at[slot]).wait()

        xcp = [pltpu.make_async_copy(s, xb.at[i], xsem.at[i]) for i, s in enumerate((ax, bx))]
        wcp = [pltpu.make_async_copy(s, wq.at[i], wsem.at[i]) for i, s in enumerate((awq, bwq))]
        wcp += [pltpu.make_async_copy(s, wo.at[i], wsem.at[2 + i]) for i, s in enumerate((awo, bwo))]
        for c in xcp + wcp:
            c.start()
        if dma:
            for t in range(P):
                kv_start(t, t, pattern)
        acc[...] = jnp.zeros(acc.shape, F32)
        for c in xcp + wcp:
            c.wait()

        def qproj(i, t):
            g = t // B
            b = t % B
            col = pl.multiple_of(g * GW, GW) if not isinstance(g, int) else g * GW
            q = jnp.dot(xb[i, b], wq[i, :, pl.ds(col, GW)], preferred_element_type=F32)
            q = (q * (Dh ** -0.5 * LOG2E)).astype(BF16)
            for h in range(G):
                qb[i, h] = q[:, h * Dh:(h + 1) * Dh]

        qproj(0, 0)
        qproj(1, 0)

        def body(t, prefetch):
            slot = t % NSLOT
            g = t // B
            b = t % B
            if dma:
                kv_wait(slot)
            nparts = 4 * G
            parts = [pattern[len(pattern) * j // nparts: len(pattern) * (j + 1) // nparts] for j in range(nparts)]
            state = {"n": 0}
            def tick():
                if dma and prefetch and spread:
                    kv_start(t + P, (t + P) % NSLOT, parts[state["n"]])
                state["n"] += 1
            if dma and prefetch and not spread:
                kv_start(t + P, (t + P) % NSLOT, pattern)

            def qk(i, h):
                tick()
                return jax.lax.dot_general(qb[i, h], kv[slot, 2 * i, h], NT, preferred_element_type=F32)

            def pv(i, h, s):
                m = jnp.max(s, axis=-1, keepdims=True)
                p = jnp.exp2(s - m)
                l = jnp.sum(p, axis=-1, keepdims=True)
                tick()
                o = jnp.dot(p.astype(BF16), kv[slot, 2 * i + 1, h], preferred_element_type=F32)
                return (o * (1.0 / l)).astype(BF16)

            def oproj(i, os_):
                o = jnp.concatenate(os_, axis=-1)
                row = pl.multiple_of(g * GW, GW)
                r = acc[i, b] + jnp.dot(o, wo[i, pl.ds(row, GW), :], preferred_element_type=F32)
                acc[i, b] = r
                ob[b, :, i * D:(i + 1) * D] = r.astype(BF16)

            if not compute:
                for _ in range(nparts): tick()
                return
            tn = jnp.minimum(t + 1, NIT - 1)
            order = [(i, h) for i in range(2) for h in range(G)]
            outs = {0: [], 1: []}
            s_prev = qk(*order[0])
            for j in range(len(order)):
                s_next = qk(*order[j + 1]) if j + 1 < len(order) else None
                if j + 1 == len(order):
                    oproj(0, outs[0])
                outs[order[j][0]].append(pv(*order[j], s_prev))
                s_prev = s_next
            qproj(0, tn)
            oproj(1, outs[1])
            qproj(1, tn)

        jax.lax.fori_loop(0, NIT - P, lambda t, _: body(t, True), None)
        nearly = B - P
        o1 = pltpu.make_async_copy(ob.at[pl.ds(0, nearly)], out.at[pl.ds(0, nearly)], osem.at[0])
        o1.start()
        jax.lax.fori_loop(NIT - P, NIT, lambda t, _: body(t, False), None)
        o2 = pltpu.make_async_copy(ob.at[pl.ds(nearly, P)], out.at[pl.ds(nearly, P)], osem.at[1])
        o2.start()
        o1.wait()
        o2.wait()

    @jax.jit
    def f(ax, ak, av, awq, awo, bx, bk, bv, bwq, bwo):
        r = lambda a: a.reshape(B * H, Sk, Dh)
        return pl.pallas_call(
            kern,
            in_specs=[pl.BlockSpec(memory_space=pl.ANY)] * 10,
            out_specs=pl.BlockSpec(memory_space=pl.ANY),
            out_shape=jax.ShapeDtypeStruct((B, Sq, 2 * D), BF16),
            scratch_shapes=[
                pltpu.VMEM((NSLOT, 4, G, Sk, Dh), BF16),
                pltpu.VMEM((2, B, Sq, D), BF16),
                pltpu.VMEM((2, D, H * Dh), BF16),
                pltpu.VMEM((2, H * Dh, D), BF16),
                pltpu.VMEM((2, G, Sq, Dh), BF16),
                pltpu.VMEM((2, B, Sq, D), F32),
                pltpu.VMEM((B, Sq, 2 * D), BF16),
                pltpu.SemaphoreType.DMA((NSLOT,)),
                pltpu.SemaphoreType.DMA((2,)),
                pltpu.SemaphoreType.DMA((4,)),
                pltpu.SemaphoreType.DMA((2,)),
            ],
            compiler_params=pltpu.CompilerParams(vmem_limit_bytes=110 * 2**20, disable_bounds_checks=True, flags=flags),
            name="attn_v1",
        )(ax, r(ak), r(av), awq, awo, bx, r(bk), r(bv), bwq, bwo)
    return f


_impl = make(rows=1024)

@jax.jit
def pallas_concat_heads__mha_block_cached__gqa_block_cached__near_ridge_kernel(
    A_x, A_k_cache, A_v_cache, A_wq, A_wo, B_x, B_k_cache, B_v_cache, B_wq, B_wo):
    return _impl(A_x, A_k_cache, A_v_cache, A_wq, A_wo, B_x, B_k_cache, B_v_cache, B_wq, B_wo)
```

```python
import functools, itertools
import jax, jax.numpy as jnp, numpy as np
from jax.experimental import pallas as pl
from jax.experimental.pallas import tpu as pltpu

B, Sq, D, H, Sk, Dh = 16, 160, 512, 32, 1024, 128
QSCALE = Dh ** -0.5 * 1.4426950408889634
F32, BF16, U32 = jnp.float32, jnp.bfloat16, jnp.uint32
NT = (((1,), (1,)), ((), ()))
G = 4
NG = H // G
NIT = NG * B
CH = 128
NCH = Sk // CH

def mo(x, m):
    return x if isinstance(x, int) else pl.multiple_of(x, m)

def lin(cols):
    out = []
    for n in range(1 << len(cols)):
        y = 0
        for k, c in enumerate(cols):
            if n >> k & 1: y ^= c
        out.append(y)
    return out

SCHED0 = 'o4 o5 s0 e0 s1 e1 p0 o6 q2 s2 e2 p1 q3 s3 e3 q4 o7 p2 s4 e4 q5 p3 q6 s5 p4 o0 e5 o1 s6 e6 o2 q7 p5 s7 e7 o3 p6 q1 p7'

def make(sched=SCHED0, NSLOT=4, dma=True, compute=True, flags=None, cols=(32, 16, 24, 88, 1, 2, 4), lead=96,
         rsplit=10, tickmode="sp", aux=True, full="kv", delay=0, o4=(0, 2, 3, 1), wtick=None, wr=True, wch=16, pstore=False, smax="a"):
    ops = sched.split()
    pattern = [(y >> 5, (y >> 3) & 3, y & 7, n % 2) for n, y in enumerate(lin(cols))]
    pre = [j for j in range(G) if f"q{j}" not in ops]
    assert pre == list(range(len(pre)))
    NP = len(pre)

    def kern(ax, ak, av, awq, awo, bx, bk, bv, bwq, bwo, out,
             kv, xb, wq, wo, q0, qb, oh, acc, ob, kvsem, asem, osem, *pb):
        xs, srcs, wqs, wos = (ax, bx), (ak, av, bk, bv), (awq, bwq), (awo, bwo)

        def kv_start(t, part):
            slot = t & (NSLOT - 1)
            base = ((t >> 2) * 16 + (t & 3)) * NCH
            for a, k, c, prio in part:
                pltpu.make_async_copy(srcs[a].at[base + (k * 4 * NCH) + c], kv.at[slot, a, k, pl.ds(mo(c * CH, CH), CH)],
                                      kvsem.at[slot]).start(priority=prio)

        def kv_wait(t):
            slot = t & (NSLOT - 1)
            pltpu.make_async_copy(kv.at[slot], kv.at[slot], kvsem.at[slot]).wait()

        def wq_start(i, s, c, half, prio, sem):
            r, l = pl.ds(mo(s * 128 + c * 8, 8), 8), pl.ds(mo(half * 2048, 2048), 2048)
            pltpu.make_async_copy(wqs[i].at[r, l], wq.at[i, half, r], asem.at[sem]).start(priority=prio)

        def wo_start(i, s, c, prio):
            g = (s >> 1) * 4 + ((c >> 2) & 3)
            r = (((s & 1) * 2 + (c >> 4)) * 4 + (c & 3)) * 32
            pltpu.make_async_copy(wos[i].at[pl.ds(mo(s * 1024 + c * 32, 32), 32)], wo.at[i, g, pl.ds(mo(r, 32), 32)],
                                  asem.at[3]).start(priority=prio)

        def x_start(i, s, c, prio):
            r = pl.ds(mo(s * 512 + c * 32, 32), 32)
            pltpu.make_async_copy(xs[i].at[r], xb.at[i, r], asem.at[4 + i]).start(priority=prio)

        def wait(buf, k):
            pltpu.make_async_copy(buf, buf, asem.at[k]).wait()

        kv32 = kv.bitcast(U32)
        def unpack(w):
            return pltpu.bitcast(w, BF16)
        def pack(v):
            return pltpu.bitcast(v.astype(BF16), U32)

        if aux:
            @pl.loop(0, 2)
            def _(i):
                @pl.loop(0, 16)
                def _(c):
                    for n, s in enumerate(o4):
                        wq_start(0, s, c, i, 0, i)
                        for u in range(2):
                            pl.when(i == u)(functools.partial(x_start, u, s, c, 1))
                    for u in range(2):
                        pl.when(i == u)(functools.partial(x_start, u, 4, c, u))
                    @pl.when(jnp.logical_and(i == 1, c == 10))
                    def _():
                        wait(wq.at[0, 0], 0)
                        wait(xb.at[0], 4)
            def aux2(c):
                for n, s in enumerate(o4):
                    wo_start(0, s, c, 0)
                    wo_start(1, s, c, 1)
                for n, s in enumerate(o4):
                    wq_start(1, s, c >> 1, c & 1, n % 2, 2)
        nkv = NCH + lead // 16
        @pl.loop(0, 16)
        def _(u):
            if aux:
                pl.when(u == 8)(lambda: wait(wq.at[0, 1], 1))
            for v in range(3):
                w = 3 * u + v
                if aux:
                    pl.when(w < 32)(functools.partial(aux2, w))
                if dma:
                    @pl.when(jnp.logical_and(w >= 32, w < 32 + nkv))
                    def _():
                        kv_start((w - 32) >> 3, [(a, k, w & 7, prio) for a, k, c, prio in pattern[:16]])
            if NP and compute:
                b2, g1 = u & 7, u >> 3
                q = jnp.dot(xb[0, pl.ds(mo(b2 * 2 * Sq, 2 * Sq), 2 * Sq)], wq[0, g1, :, :NP * 4 * Dh], preferred_element_type=F32)
                for bb in range(2):
                    for n in range(NP * 4):
                        q0[(b2 * 2 + bb) * NG + g1 * 4 + n % 4, n // 4] = pack(q[bb * Sq:(bb + 1) * Sq, n * Dh:(n + 1) * Dh] * QSCALE)
        assert lead % 16 == 0
        assert sorted((a, k, c) for a, k, c, _ in pattern[:lead]) == sorted((a, k, c) for a in range(4) for k in range(4) for c in range(lead // 16))
        oh[...] = jnp.zeros(oh.shape, U32)
        acc[...] = jnp.zeros(acc.shape, F32)
        if aux:
            wait(wq.at[1], 2)
            wait(wo, 3)
            wait(xb.at[1], 5)

        def qproj(j, t):
            i, k = divmod(j, G)
            col = mo(((t & 3) + 4 * k) * Dh, Dh)
            q = jnp.dot(xb[i, pl.ds(mo((t >> 3) * Sq, Sq), Sq)], wq[i, (t >> 2) & 1, :, pl.ds(col, Dh)], preferred_element_type=F32)
            qb[j] = pack(q * QSCALE)

        def oproj(j, g, b):
            i, n = divmod(j, G)
            r = jnp.dot(unpack(oh[i]), wo[i, g, :, n * Dh:(n + 1) * Dh], preferred_element_type=F32)
            r = r + jnp.where(g == 0, 0.0, acc[j])
            acc[j] = r
            ob[b, :, j * Dh:(j + 1) * Dh] = r.astype(BF16)

        pos = {op: k for k, op in enumerate(ops)}
        carried_q = [j for j in range(2 * G) if f"q{j}" in pos and pos[f"q{j}"] > pos[f"s{j}"]]
        late_o = [j for j in range(2 * G) if pos[f"o{j}"] < min(pos[f"p{(j // G) * G + h}"] for h in range(G))]
        for j in range(2 * G):
            assert j in late_o or pos[f"o{j}"] > max(pos[f"p{(j // G) * G + h}"] for h in range(G))
            assert pos[f"s{j}"] < pos[f"e{j}"] < pos[f"p{j}"]
        if compute:
            for j in carried_q:
                qproj(j, 0)
        if dma:
            kv_wait(0)

        def out_start():
            for r0 in range(0, Sq, wch):
                r = pl.ds(r0, min(wch, Sq - r0))
                pltpu.make_async_copy(ob.at[pl.ds(0, B - 1), r], out.at[pl.ds(0, B - 1), r], osem.at[0]).start()

        @pl.loop(0, NIT)
        def body(t):
            tn = jnp.minimum(t + 1, NIT - 1)
            slot = t & (NSLOT - 1)
            seq = [(1, p) for p in pattern[lead:]] + [(2, p) for p in pattern[:lead]]
            nt = sum(op[0] in tickmode for op in ops)
            wt = nt * (len(seq) - lead) // len(seq) if wtick is None else wtick
            state = {"n": 0}
            def tick():
                k = state["n"]
                state["n"] += 1
                if k == wt and wr:
                    pl.when(t == NIT - 2)(out_start)
                if not dma: return
                part = seq[len(seq) * k // nt: len(seq) * (k + 1) // nt]
                for dt, grp in itertools.groupby(part, key=lambda z: z[0]):
                    pl.when(t + dt < NIT)(functools.partial(kv_start, t + dt, [z[1] for z in grp]))
            s, rl, pp = {}, {}, {}
            for op in ops:
                kind, j = op[0], int(op[1:] or 0)
                i, h = divmod(j, G)
                if kind in tickmode:
                    tick()
                if not compute:
                    if delay and kind in tickmode: pl.delay(delay)
                    continue
                if kind == "q":
                    qproj(j, tn if j in carried_q else t)
                elif kind == "o":
                    if j in late_o:
                        oproj(j, (t - 1) & (NG - 1), jnp.maximum(t - 1, 0) >> 3)
                    else:
                        oproj(j, t & (NG - 1), t >> 3)
                elif kind == "s":
                    k = unpack(kv32[slot, 2 * i, h]) if "k" in full else kv[slot, 2 * i, h]
                    s[j] = jax.lax.dot_general(unpack(q0[t, j] if j in pre else qb[j]), k, NT, preferred_element_type=F32)
                elif kind == "e":
                    ps, rs = [], []
                    for r0 in range(0, Sq, Sq // rsplit):
                        sj = s[j][r0:r0 + Sq // rsplit]
                        m = jnp.max(sj, axis=-1, keepdims=True)
                        p = jnp.exp2(sj - m)
                        if pstore:
                            pb[j % 2][r0 // 2:(r0 + Sq // rsplit) // 2] = pack(p)
                        ps.append(p.astype(BF16))
                        l = jnp.sum(p, axis=-1, keepdims=True)
                        r = pltpu.reciprocal(l, approx=True)
                        rs.append(r + r * (1.0 - l * r))
                    rl[j] = jnp.concatenate(rs, axis=0)
                    pp[j] = jnp.concatenate(ps, axis=0)
                elif kind == "p":
                    v = unpack(kv32[slot, 2 * i + 1, h]) if "v" in full else kv[slot, 2 * i + 1, h]
                    o = jnp.dot(unpack(pb[j % 2][...]) if pstore else pp[j], v, preferred_element_type=F32)
                    oh[i, :, h * Dh:(h + 1) * Dh] = pack(o * rl[j])
            if dma:
                pl.when(t + 1 < NIT)(lambda: kv_wait(t + 1))

        if wr:
            tail = [pltpu.make_async_copy(ob.at[B - 1, :, pl.ds(i * D, D)], out.at[B - 1, :, pl.ds(i * D, D)], osem.at[1 + i]) for i in range(2)]
            for i, c in enumerate(tail):
                if compute:
                    for j in late_o:
                        if j // G == i:
                            oproj(j, NG - 1, B - 1)
                c.start()
            r = pl.ds(0, B - 1)
            pltpu.make_async_copy(ob.at[r], out.at[r], osem.at[0]).wait()
            for c in tail:
                c.wait()

    @jax.jit
    def f(ax, ak, av, awq, awo, bx, bk, bv, bwq, bwo):
        r = lambda a: a.reshape(-1, CH, Dh)
        rx = lambda a: a.reshape(B * Sq, D)
        return pl.pallas_call(
            kern,
            in_specs=[pl.BlockSpec(memory_space=pl.ANY)] * 10,
            out_specs=pl.BlockSpec(memory_space=pl.ANY),
            out_shape=jax.ShapeDtypeStruct((B, Sq, 2 * D), BF16),
            scratch_shapes=[
                pltpu.VMEM((NSLOT, 4, G, Sk, Dh), BF16),
                pltpu.VMEM((2, B * Sq, D), BF16),
                pltpu.VMEM((2, 2, D, H * Dh // 2), BF16),
                pltpu.VMEM((2, NG, G * Dh, D), BF16),
                pltpu.VMEM((NIT, max(NP, 1), Sq // 2, Dh), U32),
                pltpu.VMEM((2 * G, Sq // 2, Dh), U32),
                pltpu.VMEM((2, Sq // 2, G * Dh), U32),
                pltpu.VMEM((2 * G, Sq, Dh), F32),
                pltpu.VMEM((B, Sq, 2 * D), BF16),
                pltpu.SemaphoreType.DMA((NSLOT,)),
                pltpu.SemaphoreType.DMA((6,)),
                pltpu.SemaphoreType.DMA((3,)),
            ] + [pltpu.VMEM((Sq // 2, Sk), U32)] * (2 if pstore else 0),
            compiler_params=pltpu.CompilerParams(vmem_limit_bytes=110 * 2**20, disable_bounds_checks=True, flags=flags),
            name="attn_v7",
        )(rx(ax), r(ak), r(av), awq, awo, rx(bx), r(bk), r(bv), bwq, bwo)
    return f

def co(**kw):
    return make(dma=False, aux=False, **kw)
def do(**kw):
    return make(compute=False, **kw)
S2 = 'o4 o5 s0 e0 s1 e1 p0 o6 q2 s2 e2 p1 q3 s3 e3 q4 o7 p2 s4 e4 q5 p3 q6 s5 p4 o0 e5 o1 s6 e6 o2 q7 p5 s7 e7 p6 o3 p7'


_impl = make(wtick=11)

@jax.jit
def pallas_concat_heads__mha_block_cached__gqa_block_cached__near_ridge_kernel(
    A_x, A_k_cache, A_v_cache, A_wq, A_wo, B_x, B_k_cache, B_v_cache, B_wq, B_wo):
    return _impl(A_x, A_k_cache, A_v_cache, A_wq, A_wo, B_x, B_k_cache, B_v_cache, B_wq, B_wo)
```

```python
import functools

import jax
import jax.numpy as jnp
import jax.experimental.pallas as pl
import jax.experimental.pallas.tpu as pltpu

F32, BF16, U32 = jnp.float32, jnp.bfloat16, jnp.uint32

B, SQ, D, H, SK, DH = 16, 160, 512, 32, 1024, 128
G = 4
NG = H // G
STEPS = B * NG
NSLOT = 4
CH = 128
NCH = SK // CH
Q_SCALE = DH ** -0.5 * 1.4426950408889634

STREAMS = (0, 2, 3, 1, 5, 6, 4, 7)
QUARTERS = (0, 2, 3, 1)
LEAD = (4, 6)
EARLY_Q = (SQ, 48)
SCHEDULE = ("o4 o5 s0 e0 s1 e1 o6 p0 q2 s2 e2 p1 q3 s3 e3 q4 o7 p2 s4 e4 "
            "q5 s5 p3 q6 p4 o1 e5 o0 s6 p5 o2 e6 q7 s7 e7 o3 p6 q1 p7")
WRITE_AT = 13


def _pack(x):
    return pltpu.bitcast(x.astype(BF16), U32)


def _unpack(x):
    return pltpu.bitcast(x, BF16)


def _ds(start, size, align):
    if not isinstance(start, int):
        start = pl.multiple_of(start, align)
    return pl.ds(start, size)


def _softmax(s):
    ps, inv = [], []
    for r in range(0, SQ, 16):
        p = jnp.exp2(s[r:r + 16] - jnp.max(s[r:r + 16], axis=1, keepdims=True))
        ps.append(p.astype(BF16))
        inv.append(pltpu.reciprocal(jnp.sum(p, axis=1, keepdims=True), full_range=False))
    return jnp.concatenate(ps, axis=0), jnp.concatenate(inv, axis=0)


def _kernel(a_x, a_k, a_v, a_wq, a_wo, b_x, b_k, b_v, b_wq, b_wo, out,
            kv, x, wq_a, wq_b, wo, q_early, q, o, acc, res,
            kv_sem, in_sem, out_sem):
    wq = (wq_a, wq_b)

    def kv_start(is_v, t, c, j):
        c = (c & 4) | ((c & 1) << 1) | ((c >> 1) & 1)
        rows = _ds(c * CH, CH, CH)
        slot = t & (NSLOT - 1)
        cache = ((a_k, b_k), (a_v, b_v))[is_v][j // G]
        pltpu.make_async_copy(
            cache.at[(t >> 2) * 16 + (t & 3) + 4 * (j % G), rows],
            kv.at[slot, is_v, j, rows], kv_sem.at[slot]).start(priority=is_v)

    def kv_round(n):
        for j in STREAMS:
            for is_v in range(2):
                m = n + LEAD[is_v] - LEAD[1]
                pl.when(m >= 0)(functools.partial(kv_start, is_v, m >> 3, m & 7, j))

    def kv_wait(t):
        slot = t & (NSLOT - 1)
        pltpu.make_async_copy(kv.at[slot], kv.at[slot], kv_sem.at[slot]).wait()

    def wq_start(i, s, c, priority):
        rows = _ds(s * 128 + (c >> 1) * 8, 8, 8)
        cols = _ds((c & 1) * 2048, 2048, 2048)
        pltpu.make_async_copy((a_wq, b_wq)[i].at[rows, cols], wq[i].at[rows, cols],
                              in_sem.at[i]).start(priority=priority)

    def wo_start(i, s, c):
        g = (s >> 1) * 4 + ((c >> 2) & 3)
        row = (((s & 1) * 2 + (c >> 4)) * 4 + (c & 3)) * 32
        pltpu.make_async_copy((a_wo, b_wo)[i].at[_ds(s * 1024 + c * 32, 32, 32)],
                              wo.at[i, g, _ds(row, 32, 32)],
                              in_sem.at[2]).start(priority=i)

    def x_start(i, s, c, priority):
        rows = _ds(s * 512 + c * 32, 32, 32)
        pltpu.make_async_copy((a_x, b_x)[i].at[rows], x.at[i, rows],
                              in_sem.at[3]).start(priority=priority)

    def in_wait(buf, n):
        pltpu.make_async_copy(buf, buf, in_sem.at[n]).wait()

    @pl.loop(0, 16)
    def _(c):
        for i in range(2):
            for s in QUARTERS:
                wq_start(0, s, 2 * c + i, 0)
                x_start(i, s, c, 1)
        for i in range(2):
            x_start(i, 4, c, i)

    pl.loop(0, LEAD[1])(kv_round)

    @pl.loop(0, 2 * G)
    def _(j):
        acc[j] = jnp.zeros((SQ, DH), F32)
        o[j] = jnp.zeros((SQ // 2, DH), U32)

    in_wait(wq_a, 0)
    in_wait(x, 3)

    @pl.loop(0, B)
    def _(b):
        @pl.when(b < 12)
        def _():
            @pl.loop((8 * b) // 3, (8 * b + 8) // 3)
            def _(c):
                for s in QUARTERS:
                    wo_start(0, s, c)
                    wo_start(1, s, c)
                for n, s in enumerate(QUARTERS):
                    wq_start(1, s, c, n % 2)

        @pl.when(b >= 12)
        def _():
            for n in range(2):
                kv_round(LEAD[1] + 2 * b - 24 + n)

        for j, rows in enumerate(EARLY_Q):
            for half in range(2):
                head = 16 * half + 4 * j
                r = jnp.dot(x[0, _ds(b * SQ, rows, SQ)], wq_a[:, head * DH:(head + 4) * DH],
                            preferred_element_type=F32) * Q_SCALE
                for n in range(4):
                    q_early[b * NG + 4 * half + n, j, :rows // 2] = _pack(r[:, n * DH:(n + 1) * DH])

    in_wait(wq_b, 1)
    in_wait(wo, 2)

    def q_proj(j, t):
        done = EARLY_Q[j] if j < len(EARLY_Q) else 0
        head = ((t >> 2) & 1) * 16 + (t & 3) + 4 * (j % G)
        w = wq[j // G][:, _ds(head * DH, DH, DH)]
        rows = x[j // G, _ds((t >> 3) * SQ + done, SQ - done, 16)]
        q[j, done // 2:] = _pack(jnp.dot(rows, w, preferred_element_type=F32) * Q_SCALE)

    def q_load(j, t):
        done = EARLY_Q[j] if j < len(EARLY_Q) else 0
        parts = []
        if done > 0:
            parts.append(q_early[t, j, :done // 2])
        if done < SQ:
            parts.append(q[j, done // 2:])
        return _unpack(jnp.concatenate(parts, axis=0))

    def out_proj(j, g, b):
        i, n = divmod(j, G)
        heads = _unpack(jnp.concatenate([o[i * G + k] for k in range(G)], axis=1))
        r = jnp.dot(heads, wo[i, g, :, n * DH:(n + 1) * DH], preferred_element_type=F32)
        r = r + jnp.where(g == 0, 0.0, acc[j])
        acc[j] = r
        res[b, :, j * DH:(j + 1) * DH] = r.astype(BF16)

    def out_copy(rows):
        done = pl.ds(0, B - 1)
        return pltpu.make_async_copy(res.at[done, rows], out.at[done, rows], out_sem.at[0])

    def prefetch(t, n):
        if n in (WRITE_AT, WRITE_AT + 1):
            @pl.when(t == STEPS - 2)
            def _():
                for r in range(0, SQ // 2, 8):
                    out_copy(pl.ds((n - WRITE_AT) * (SQ // 2) + r, 8)).start()

        for j in STREAMS[n % 2 * 4:n % 2 * 4 + 4]:
            for is_v in range(2):
                ahead, c = divmod(NCH + LEAD[is_v] + n // 2, NCH)
                pl.when(t + ahead < STEPS)(functools.partial(kv_start, is_v, t + ahead, c, j))

    q_proj(1, 0)
    kv_wait(0)

    @pl.loop(0, STEPS)
    def _(t):
        slot = t & (NSLOT - 1)
        live, part = {}, 0
        for op in SCHEDULE.split():
            kind, j = op[0], int(op[1])
            if kind in "sp":
                prefetch(t, part)
                part += 1
            if kind == "q":
                q_proj(j, jnp.minimum(t + 1, STEPS - 1) if j == 1 else t)
            elif kind == "s":
                live[j] = jax.lax.dot_general(
                    q_load(j, t), kv[slot, 0, j], (((1,), (1,)), ((), ())),
                    preferred_element_type=F32)
            elif kind == "e":
                live[j] = _softmax(live[j])
            elif kind == "p":
                p, inv = live.pop(j)
                o[j] = _pack(jnp.dot(p, kv[slot, 1, j], preferred_element_type=F32) * inv)
            elif j >= G:
                out_proj(j, (t - 1) & (NG - 1), jnp.maximum(t - 1, 0) >> 3)
            else:
                out_proj(j, t & (NG - 1), t >> 3)
        pl.when(t + 1 < STEPS)(functools.partial(kv_wait, t + 1))

    last = [pltpu.make_async_copy(res.at[B - 1, :, pl.ds(i * D, D)],
                                  out.at[B - 1, :, pl.ds(i * D, D)], out_sem.at[1 + i])
            for i in range(2)]
    last[0].start()
    for j in range(G, 2 * G):
        out_proj(j, NG - 1, B - 1)
    last[1].start()
    out_copy(pl.ds(0, SQ)).wait()
    last[0].wait()
    last[1].wait()


@jax.jit
def pallas_concat_heads__mha_block_cached__gqa_block_cached__near_ridge_kernel(
    A_x: jax.Array,
    A_k_cache: jax.Array,
    A_v_cache: jax.Array,
    A_wq: jax.Array,
    A_wo: jax.Array,
    B_x: jax.Array,
    B_k_cache: jax.Array,
    B_v_cache: jax.Array,
    B_wq: jax.Array,
    B_wo: jax.Array,
):
    assert A_x.shape == B_x.shape == (B, SQ, D)
    assert A_k_cache.shape == A_v_cache.shape == (B, H, SK, DH)
    assert B_k_cache.shape == B_v_cache.shape == (B, H, SK, DH)
    rows = lambda a: a.reshape(B * SQ, D)
    heads = lambda a: a.reshape(B * H, SK, DH)
    return pl.pallas_call(
        _kernel,
        in_specs=[pl.BlockSpec(memory_space=pl.ANY)] * 10,
        out_specs=pl.BlockSpec(memory_space=pl.ANY),
        out_shape=jax.ShapeDtypeStruct((B, SQ, 2 * D), BF16),
        scratch_shapes=[
            pltpu.VMEM((NSLOT, 2, 2 * G, SK, DH), BF16),
            pltpu.VMEM((2, B * SQ, D), BF16),
            pltpu.VMEM((D, H * DH), BF16),
            pltpu.VMEM((D, H * DH), BF16),
            pltpu.VMEM((2, NG, G * DH, D), BF16),
            pltpu.VMEM((STEPS, len(EARLY_Q), SQ // 2, DH), U32),
            pltpu.VMEM((2 * G, SQ // 2, DH), U32),
            pltpu.VMEM((2 * G, SQ // 2, DH), U32),
            pltpu.VMEM((2 * G, SQ, DH), F32),
            pltpu.VMEM((B, SQ, 2 * D), BF16),
            pltpu.SemaphoreType.DMA((NSLOT,)),
            pltpu.SemaphoreType.DMA((4,)),
            pltpu.SemaphoreType.DMA((3,)),
        ],
        compiler_params=pltpu.CompilerParams(
            vmem_limit_bytes=80 * 2**20, disable_bounds_checks=True),
    )(rows(A_x), heads(A_k_cache), heads(A_v_cache), A_wq, A_wo,
      rows(B_x), heads(B_k_cache), heads(B_v_cache), B_wq, B_wo)
```
